```python
import jax
import jax.numpy as jnp

def _softmax(x, axis=-1):
    return jax.nn.softmax(x, axis=axis)
def _gelu(x):
    return jax.nn.gelu(x, approximate=True)
def _silu(x):
    return jax.nn.silu(x)
def _sigmoid(x):
    return jax.nn.sigmoid(x)
def _layernorm(x, axis=-1, eps=1e-5):
    m = jnp.mean(x, axis=axis, keepdims=True)
    v = jnp.var(x, axis=axis, keepdims=True)
    return (x - m) / jnp.sqrt(v + eps)
def _scatter_add(tgt, idx, src, axis=0):
    return tgt.at[idx].add(src)
def _segment_sum(src, seg, n):
    return jax.ops.segment_sum(src, seg, n)
class _Rng:
    def __init__(self, key):
        self._k = key
    def _next(self):
        self._k, sub = jax.random.split(self._k)
        return sub
    def normal(self, shape):
        return jax.random.normal(self._next(), shape, dtype=jnp.bfloat16)
    def randint(self, lo, hi, shape):
        return jax.random.randint(self._next(), shape, lo, hi, dtype=jnp.int32)
    def uniform(self, shape, lo=0.0, hi=1.0):
        return jax.random.uniform(self._next(), shape, jnp.bfloat16, lo, hi)
    def permutation(self, n):
        return jax.random.permutation(self._next(), n)


kernel_name = 'recurrent_scan__mha_block_cached__moe_arch_mod__decode'

def setup_inputs():
    _rng = _Rng(jax.random.key(int.from_bytes(__import__("os").urandom(4), "little")))
    _w = (lambda a: (lambda t: t.astype(jnp.bfloat16) if jnp.issubdtype(t.dtype, jnp.floating) else t)(jnp.asarray(a)))
    def _A_setup():
        B, Sq, D = 2, 1, 512
        H, Sk, Dh = 32, 16384, 128
        return {
            "x": _w((lambda *s: _rng.normal(s) * 0.05)(B, Sq, D)),
            "k_cache": _w((lambda *s: _rng.normal(s) * 0.05)(B, H, Sk, Dh)),
            "v_cache": _w((lambda *s: _rng.normal(s) * 0.05)(B, H, Sk, Dh)),
            "wq": _w((lambda *s: _rng.normal(s) * 0.05)(D, H * Dh) * (D ** -0.5)),
            "wo": _w((lambda *s: _rng.normal(s) * 0.05)(H * Dh, D) * ((H * Dh) ** -0.5)),
        }
    _A_in = _A_setup()

    def _B_setup():
        B, S, D, F, C = 2, 1, 512, 1792, 1
        return {
            "x": _w((lambda *s: _rng.normal(s) * 0.05)(B, S, D)),
            "w_r": _w((lambda *s: _rng.normal(s) * 0.05)(D)),
            "w_gate": _w((lambda *s: _rng.normal(s) * 0.05)(D, F)),
            "w_up": _w((lambda *s: _rng.normal(s) * 0.05)(D, F)),
            "w_down": _w((lambda *s: _rng.normal(s) * 0.05)(F, D)),
        }
    _B_in = _B_setup()

    return {
        "A_x": _A_in["x"],
        "A_k_cache": _A_in["k_cache"],
        "A_v_cache": _A_in["v_cache"],
        "A_wq": _A_in["wq"],
        "A_wo": _A_in["wo"],
        "B_x": _B_in["x"],
        "B_w_r": _B_in["w_r"],
        "B_w_gate": _B_in["w_gate"],
        "B_w_up": _B_in["w_up"],
        "B_w_down": _B_in["w_down"],
    }

def reference(A_x, A_k_cache, A_v_cache, A_wq, A_wo, B_x, B_w_r, B_w_gate, B_w_up, B_w_down):
    def _A_ref(x, k_cache, v_cache, wq, wo):
        B, Sq, D = x.shape
        H, Dh = 32, 128
        q = (lambda x, *d: x.transpose(*d))((x @ wq).reshape(B, Sq, H, Dh), 0, 2, 1, 3)
        scores = jnp.einsum("bhqd,bhkd->bhqk", q, k_cache) * (Dh ** -0.5)
        p = _softmax(scores, axis=-1)
        o = jnp.einsum("bhqk,bhkd->bhqd", p, v_cache)
        return (lambda x, *d: x.transpose(*d))(o, 0, 2, 1, 3).reshape(B, Sq, H * Dh) @ wo

    def _B_ref(x, w_r, w_gate, w_up, w_down):
        B, S, D = x.shape
        C = 1
        r = x @ w_r
        idx = jnp.argsort(-r, axis=-1)[:, :C]
        idx_e = jnp.repeat(idx.reshape(B, C, 1), D, axis=2)
        x_sel = jnp.take_along_axis(x, idx_e, axis=1)
        g = _silu(x_sel @ w_gate)
        u = x_sel @ w_up
        y = (g * u) @ w_down
        r_sel = _sigmoid(jnp.take_along_axis(r, idx, axis=1))
        y = y * r_sel.reshape(B, C, 1)
        b_off = (jnp.arange(B) * S).reshape(B, 1)
        flat_idx = (idx + b_off).reshape(B * C)
        zero = (x * 0.0).reshape(B * S, D)
        upd = _scatter_add(zero, flat_idx, y.reshape(B * C, D), axis=0)
        return x + upd.reshape(B, S, D)

    x = A_x
    xn = _layernorm(x, axis=-1)
    s = _A_ref(xn, A_k_cache, A_v_cache, A_wq, A_wo)
    g = _silu(_B_ref(xn, B_w_r, B_w_gate, B_w_up, B_w_down))
    return x + s * g
```

```python
import functools

import jax
import jax.numpy as jnp
import jax.experimental.pallas as pl
import jax.experimental.pallas.tpu as pltpu

F32 = jnp.float32
BF16 = jnp.bfloat16


def _splits(n_rows, n):
    u = n_rows // 16
    b = [(u * i) // n * 16 for i in range(n + 1)]
    return [(b[i], b[i + 1] - b[i]) for i in range(n)]


def _make(CH=2048, NP=10, LOOK=5, SUB=256, prios=(0, 1)):
    NSLOT = LOOK + 1

    def kernel(x_hbm, k_hbm, v_hbm, wq_hbm, wo_hbm, wr_hbm, wg_hbm, wu_hbm, wd_hbm,
               o_ref,
               x_v, wr_v, wq_v, wo_v, wg_v, wu_v, wd_v, kbuf, vbuf,
               xn_s, s_acc, g_s, kv_sem, w_sem):
        B, H, S, Dh = k_hbm.shape
        D = x_hbm.shape[-1]
        nch = S // CH
        total = B * H * nch
        pieces = _splits(CH, NP)
        scale = Dh ** -0.5

        def start_pair(i, slot, j):
            t = i // nch
            b, h, c = t // H, t % H, i % nch
            off, n = pieces[j]
            r0 = pl.multiple_of(c * CH + off, 16)
            pltpu.make_async_copy(k_hbm.at[b, h, pl.ds(r0, n)], kbuf.at[slot, pl.ds(off, n)],
                                  kv_sem.at[0, slot]).start(priority=prios[0])
            pltpu.make_async_copy(v_hbm.at[b, h, pl.ds(r0, n)], vbuf.at[slot, pl.ds(off, n)],
                                  kv_sem.at[1, slot]).start(priority=prios[1])

        def start_chunk(i, slot):
            for j in range(NP):
                start_pair(i, slot, j)

        def stream_weight(src, dst, sem, rows, cols):
            R, C = src.shape
            ncol = len(cols)

            def body(r, _):
                for c0, cn in cols:
                    for half in range(2):
                        r0 = pl.multiple_of(half * (R // 2) + r * rows, 16)
                        pltpu.make_async_copy(
                            src.at[pl.ds(r0, rows), pl.ds(c0, cn)],
                            dst.at[pl.ds(r0, rows), pl.ds(c0, cn)], sem).start(priority=prios[half])
            jax.lax.fori_loop(0, R // 2 // rows, body, None)

        def wait_all(dst, sem):
            pltpu.make_async_copy(dst, dst, sem).wait()

        cx = pltpu.make_async_copy(x_hbm, x_v, w_sem.at[0])
        cr = pltpu.make_async_copy(wr_hbm, wr_v, w_sem.at[1])
        cx.start()
        cr.start()
        stream_weight(wg_hbm, wg_v, w_sem.at[2], 16, [(0, 896), (896, 896)])
        stream_weight(wu_hbm, wu_v, w_sem.at[3], 16, [(0, 896), (896, 896)])
        stream_weight(wd_hbm, wd_v, w_sem.at[4], 32, [(0, 512)])
        stream_weight(wq_hbm, wq_v, w_sem.at[5], 16, [(0, 1408), (1408, 1280), (2688, 1408)])
        stream_weight(wo_hbm, wo_v, w_sem.at[6], 32, [(0, 512)])
        start_chunk(0, 0)

        cx.wait()
        cr.wait()
        wr = wr_v[...].astype(F32).reshape(1, D)
        rows = jax.lax.broadcasted_iota(jnp.int32, (16, D), 0)
        x32 = x_v[...].astype(F32)
        xs = [jnp.broadcast_to(x32[b:b + 1], (16, D)) for b in range(B)]
        xns = []
        for b in range(B):
            mu = jnp.mean(xs[b], axis=-1, keepdims=True)
            xc = xs[b] - mu
            var = jnp.mean(xc * xc, axis=-1, keepdims=True)
            xn = (xc / jnp.sqrt(var + 1e-5)).astype(BF16)
            xn_s[b] = xn
            s_acc[b] = jnp.zeros((16, D), F32)
            xns.append(xn)
        xn2 = jnp.where(rows == 0, xns[0].astype(F32), xns[1].astype(F32))
        xn2b = xn2.astype(BF16)
        r = jnp.sum(xn2 * wr, axis=-1, keepdims=True)
        wait_all(wg_v, w_sem.at[2])
        g = jnp.dot(xn2b, wg_v[...], preferred_element_type=F32)
        start_chunk(1, 1)
        wait_all(wu_v, w_sem.at[3])
        u = jnp.dot(xn2b, wu_v[...], preferred_element_type=F32)
        hmid = (g * jax.nn.sigmoid(g) * u).astype(BF16)
        start_chunk(2, 2)
        wait_all(wd_v, w_sem.at[4])
        y = jnp.dot(hmid, wd_v[...], preferred_element_type=F32) * jax.nn.sigmoid(r)
        z = xn2 + (xn2 * 0.0 + y)
        g_s[...] = z * jax.nn.sigmoid(z)
        jax.lax.fori_loop(3, LOOK, lambda i, _: start_chunk(i, i), None)
        wait_all(wq_v, w_sem.at[5])
        wait_all(wo_v, w_sem.at[6])

        nsub = CH // SUB

        def chunk(i, carry, prefetch):
            q, m, l, acc = carry
            slot = i % NSLOT
            nslot = (i + LOOK) % NSLOT
            plan = [[] for _ in range(2 * nsub)]
            for j in range(NP):
                plan[(j * 2 * nsub) // NP].append(j)

            def issue(step):
                if prefetch:
                    for j in plan[step]:
                        start_pair(i + LOOK, nslot, j)

            wait_all(kbuf.at[slot], kv_sem.at[0, slot])
            wait_all(vbuf.at[slot], kv_sem.at[1, slot])
            ss = []
            for t in range(nsub):
                issue(t)
                kt = kbuf[slot, pl.ds(t * SUB, SUB), :]
                ss.append(jax.lax.dot_general(q, kt, (((1,), (1,)), ((), ())),
                                              preferred_element_type=F32) * scale)
            mx = functools.reduce(jnp.maximum, ss)
            m_new = jnp.maximum(m, jnp.max(mx, axis=-1, keepdims=True))
            alpha = jnp.exp(m - m_new)
            l = l * alpha
            acc = acc * alpha
            for t in range(nsub):
                issue(nsub + t)
                p = jnp.exp(ss[t] - m_new)
                for c in range(SUB // 128):
                    l = l + p[:, c * 128:(c + 1) * 128]
                vt = vbuf[slot, pl.ds(t * SUB, SUB), :]
                acc = acc + jnp.dot(p.astype(BF16), vt, preferred_element_type=F32)
            return q, m_new, l, acc

        M = 16

        def head_begin(t):
            b, h = t // H, t % H
            c0 = pl.multiple_of(h * Dh, Dh)
            q = jnp.dot(xn_s[b], wq_v[:, pl.ds(c0, Dh)], preferred_element_type=F32).astype(BF16)
            return (q, jnp.full((M, 1), -jnp.inf, F32), jnp.zeros((M, 128), F32), jnp.zeros((M, Dh), F32))

        def head_end(t, carry):
            b, h = t // H, t % H
            _, _, l, acc = carry
            o = (acc / jnp.sum(l, axis=-1, keepdims=True)).astype(BF16)
            r0 = pl.multiple_of(h * Dh, Dh)
            s_acc[b] += jnp.dot(o, wo_v[pl.ds(r0, Dh), :], preferred_element_type=F32)

        def head(t, _):
            carry = head_begin(t)
            carry = jax.lax.fori_loop(0, nch, lambda c, cr_: chunk(t * nch + c, cr_, True), carry)
            head_end(t, carry)

        assert LOOK <= nch
        last = B * H - 1
        jax.lax.fori_loop(0, last, head, None)
        carry = head_begin(last)
        carry = jax.lax.fori_loop(0, nch - LOOK, lambda c, cr_: chunk(last * nch + c, cr_, True), carry)
        carry = jax.lax.fori_loop(nch - LOOK, nch, lambda c, cr_: chunk(last * nch + c, cr_, False), carry)
        head_end(last, carry)

        s2 = jnp.where(rows == 0, s_acc[0], s_acc[1])
        o_ref[...] = (x_v[...].astype(F32) + (s2 * g_s[...])[0:B]).astype(o_ref.dtype)

    def fn(A_x, A_k_cache, A_v_cache, A_wq, A_wo, B_x, B_w_r, B_w_gate, B_w_up, B_w_down):
        del B_x
        B, H, S, Dh = A_k_cache.shape
        D = A_x.shape[-1]
        any_spec = pl.BlockSpec(memory_space=pl.ANY)
        return pl.pallas_call(
            kernel,
            in_specs=[any_spec] * 9,
            out_specs=pl.BlockSpec(memory_space=pltpu.VMEM),
            out_shape=jax.ShapeDtypeStruct((B, D), A_x.dtype),
            scratch_shapes=[
                pltpu.VMEM((B, D), BF16),
                pltpu.VMEM(B_w_r.shape, BF16),
                pltpu.VMEM(A_wq.shape, BF16),
                pltpu.VMEM(A_wo.shape, BF16),
                pltpu.VMEM(B_w_gate.shape, BF16),
                pltpu.VMEM(B_w_up.shape, BF16),
                pltpu.VMEM(B_w_down.shape, BF16),
                pltpu.VMEM((NSLOT, CH, Dh), BF16),
                pltpu.VMEM((NSLOT, CH, Dh), BF16),
                pltpu.VMEM((B, 16, D), BF16),
                pltpu.VMEM((B, 16, D), F32),
                pltpu.VMEM((16, D), F32),
                pltpu.SemaphoreType.DMA((2, NSLOT)),
                pltpu.SemaphoreType.DMA((7,)),
            ],
            compiler_params=pltpu.CompilerParams(vmem_limit_bytes=100 * 1024 * 1024),
        )(A_x.reshape(B, D), A_k_cache, A_v_cache, A_wq, A_wo, B_w_r, B_w_gate, B_w_up, B_w_down).reshape(A_x.shape)

    return fn


@jax.jit
def pallas_recurrent_scan__mha_block_cached__moe_arch_mod__decode_kernel(
    A_x, A_k_cache, A_v_cache, A_wq, A_wo, B_x, B_w_r, B_w_gate, B_w_up, B_w_down
):
    return _make()(A_x, A_k_cache, A_v_cache, A_wq, A_wo, B_x, B_w_r, B_w_gate, B_w_up, B_w_down)
```

```python
import functools

import jax
import jax.numpy as jnp
import jax.experimental.pallas as pl
import jax.experimental.pallas.tpu as pltpu

F32 = jnp.float32
BF16 = jnp.bfloat16

CHUNK = 4096
SUB = 256
PAIRS = 22
Q0_ROWS = 192
LOOK = 3
NSLOT = LOOK + 1
TAIL_CUTS = (10, 14)
M = 8


def _carve(sizes):
    out, off = [], 0
    for n in sizes:
        out.append((off, n))
        off += n
    return out


def _copy_plan():
    half = PAIRS // 2
    units = (CHUNK - half * Q0_ROWS) // 8
    small = [(units * (i + 1) // half - units * i // half) * 8 for i in range(half)]
    k = _carve(small + [Q0_ROWS] * half)
    v = _carve([Q0_ROWS] * half + small)
    plan = [((0, *k[j]), (1, *v[j])) for j in range(half)]
    plan += [((1, *v[j]), (0, *k[j])) for j in range(half, PAIRS)]
    ends = [min(o for o, _ in v if o >= c * SUB) for c in TAIL_CUTS] + [CHUNK]
    return plan, list(zip([0] + ends[:-1], ends))


def _kernel(x_hbm, k_hbm, v_hbm, wq_hbm, wo_hbm, wr_hbm, wg_hbm, wu_hbm, wd_hbm,
            o_ref,
            x_v, wr_v, wq_v, wo_v, wg_v, wu_v, wd_v, kbuf, vbuf,
            xn_s, s_acc, gate_s, kv_sem, aux_sem):
    B, H, S, Dh = k_hbm.shape
    D = x_hbm.shape[-1]
    nch = S // CHUNK
    total = B * H * nch
    nsub = CHUNK // SUB
    scale = Dh ** -0.5
    plan, tail_rows = _copy_plan()
    assert B == 2 and S % CHUNK == 0 and LOOK == 3 and LOOK < nch

    def tail_sem(group, slot):
        return kv_sem.at[1, slot] if group == 0 else aux_sem.at[group - 1]

    def start_pair(i, slot, j, tail=False):
        t = i // nch
        for priority, (arr, off, n) in zip((1, 0), plan[j]):
            src, dst = ((k_hbm, kbuf), (v_hbm, vbuf))[arr]
            sem = kv_sem.at[arr, slot]
            if tail and arr == 1:
                sem = tail_sem(sum(off >= end for _, end in tail_rows), slot)
            r0 = pl.multiple_of((i % nch) * CHUNK + off, 8)
            pltpu.make_async_copy(src.at[t // H, t % H, pl.ds(r0, n)],
                                  dst.at[slot, pl.ds(off, n)], sem).start(priority=priority)

    def start_chunk(i):
        for j in range(PAIRS):
            start_pair(i, i, j)

    def start_weight(src, dst, rows, cols):
        half_rows = src.shape[0] // 2

        def body(r, _):
            for c0, cn in _carve(cols):
                for half in range(2):
                    r0 = pl.multiple_of(half * half_rows + r * rows, 16)
                    pltpu.make_async_copy(
                        src.at[pl.ds(r0, rows), pl.ds(c0, cn)],
                        dst.at[pl.ds(r0, rows), pl.ds(c0, cn)],
                        aux_sem.at[0]).start(priority=half)

        jax.lax.fori_loop(0, half_rows // rows, body, None)

    def wait_filled(dst, sem):
        pltpu.make_async_copy(dst, dst, sem).wait()

    small = [pltpu.make_async_copy(x_hbm, x_v, aux_sem.at[0]),
             pltpu.make_async_copy(wr_hbm, wr_v, aux_sem.at[0])]
    for copy in small:
        copy.start()
    start_weight(wg_hbm, wg_v, 16, [896, 896])
    start_weight(wu_hbm, wu_v, 16, [896, 896])
    start_weight(wd_hbm, wd_v, 32, [512])
    start_weight(wq_hbm, wq_v, 16, [1408, 1280, 1408])
    start_weight(wo_hbm, wo_v, 32, [512])
    start_chunk(0)
    for copy in small:
        copy.wait()
    for ref in (wg_v, wu_v, wd_v, wq_v, wo_v):
        wait_filled(ref, aux_sem.at[0])

    x32 = x_v[...].astype(F32)
    xns = []
    for b in range(B):
        xb = jnp.broadcast_to(x32[b:b + 1], (M, D))
        xc = xb - jnp.mean(xb, axis=-1, keepdims=True)
        var = jnp.mean(xc * xc, axis=-1, keepdims=True)
        xns.append((xc / jnp.sqrt(var + 1e-5)).astype(BF16).astype(F32))
        xn_s[b] = xns[b]
        s_acc[b] = jnp.zeros((M, D), F32)
    first_row = jax.lax.broadcasted_iota(jnp.int32, (M, D), 0) == 0
    xn = jnp.where(first_row, xns[0], xns[1])
    r = jnp.sum(xn * wr_v[...].astype(F32).reshape(1, D), axis=-1, keepdims=True)
    g = jnp.dot(xn.astype(BF16), wg_v[...], preferred_element_type=F32)
    start_chunk(1)
    u = jnp.dot(xn.astype(BF16), wu_v[...], preferred_element_type=F32)
    mid = (g * jax.nn.sigmoid(g) * u).astype(BF16)
    start_chunk(2)
    y = jnp.dot(mid, wd_v[...], preferred_element_type=F32) * jax.nn.sigmoid(r)
    z = xn + (xn * 0.0 + y)
    gate_s[...] = z * jax.nn.sigmoid(z)

    pairs_at = [[j for j in range(PAIRS) if j * 2 * nsub // PAIRS == step]
                for step in range(2 * nsub)]

    def chunk(i, carry, prefetch=True, prefetch_tail=False, tail=False):
        q, m, l, acc = carry
        slot = i % NSLOT

        def issue(step):
            if prefetch:
                for j in pairs_at[step]:
                    start_pair(i + LOOK, (i + LOOK) % NSLOT, j, prefetch_tail)

        wait_filled(kbuf.at[slot], kv_sem.at[0, slot])
        scores = []
        for t in range(nsub):
            issue(t)
            kt = kbuf[slot, pl.ds(t * SUB, SUB), :]
            scores.append(jax.lax.dot_general(
                q, kt, (((1,), (1,)), ((), ())), preferred_element_type=F32) * scale)
        m_new = jnp.maximum(
            m, jnp.max(functools.reduce(jnp.maximum, scores), axis=-1, keepdims=True))
        m_ref = jnp.where(m_new == -jnp.inf, 0.0, m_new)
        alpha = jnp.exp(m - m_ref)
        l = l * alpha
        acc = acc * alpha
        probs = []
        for t in range(nsub):
            p = jnp.exp(scores[t] - m_ref)
            for c in range(SUB // 128):
                l = l + p[:, c * 128:(c + 1) * 128]
            probs.append(p.astype(BF16))
        if tail:
            l = 1.0 / jnp.sum(l, axis=-1, keepdims=True)
        else:
            wait_filled(vbuf.at[slot], kv_sem.at[1, slot])
        for t in range(nsub):
            issue(nsub + t)
            if tail and t in (0, *TAIL_CUTS):
                group = (0, *TAIL_CUTS).index(t)
                lo, hi = tail_rows[group]
                wait_filled(vbuf.at[slot, pl.ds(lo, hi - lo)], tail_sem(group, slot))
            vt = vbuf[slot, pl.ds(t * SUB, SUB), :]
            acc = acc + jnp.dot(probs[t], vt, preferred_element_type=F32)
        return q, m_new, l, acc

    def head_begin(t):
        c0 = pl.multiple_of((t % H) * Dh, Dh)
        q = jnp.dot(xn_s[t // H].astype(BF16), wq_v[:, pl.ds(c0, Dh)],
                    preferred_element_type=F32).astype(BF16)
        return (q, jnp.full((M, 1), -jnp.inf, F32), jnp.zeros((M, 128), F32),
                jnp.zeros((M, Dh), F32))

    def head_end(t, inv_l, acc):
        r0 = pl.multiple_of((t % H) * Dh, Dh)
        return s_acc[t // H] + jnp.dot((acc * inv_l).astype(BF16), wo_v[pl.ds(r0, Dh), :],
                                       preferred_element_type=F32)

    def head(t, _):
        _, _, l, acc = jax.lax.fori_loop(
            0, nch, lambda c, carry: chunk(t * nch + c, carry), head_begin(t))
        s_acc[t // H] = head_end(t, 1.0 / jnp.sum(l, axis=-1, keepdims=True), acc)

    last = B * H - 1
    jax.lax.fori_loop(0, last, head, None)
    carry = head_begin(last)
    for i in range(last * nch, total - 1 - LOOK):
        carry = chunk(i, carry)
    carry = chunk(total - 1 - LOOK, carry, prefetch_tail=True)
    carry = jax.lax.fori_loop(total - LOOK, total - 1,
                              functools.partial(chunk, prefetch=False), carry)
    _, _, inv_l, acc = chunk(total - 1, carry, prefetch=False, tail=True)

    s = jnp.where(first_row, s_acc[0], head_end(last, inv_l, acc))
    o_ref[...] = (x_v[...].astype(F32) + (s * gate_s[...])[0:B]).astype(o_ref.dtype)


@jax.jit
def pallas_recurrent_scan__mha_block_cached__moe_arch_mod__decode_kernel(
    A_x: jax.Array,
    A_k_cache: jax.Array,
    A_v_cache: jax.Array,
    A_wq: jax.Array,
    A_wo: jax.Array,
    B_x: jax.Array,
    B_w_r: jax.Array,
    B_w_gate: jax.Array,
    B_w_up: jax.Array,
    B_w_down: jax.Array,
):
    del B_x
    B, _, _, Dh = A_k_cache.shape
    D = A_x.shape[-1]
    out = pl.pallas_call(
        _kernel,
        in_specs=[pl.BlockSpec(memory_space=pl.ANY)] * 9,
        out_specs=pl.BlockSpec(memory_space=pltpu.VMEM),
        out_shape=jax.ShapeDtypeStruct((B, D), A_x.dtype),
        scratch_shapes=[
            pltpu.VMEM((B, D), BF16),
            pltpu.VMEM(B_w_r.shape, BF16),
            pltpu.VMEM(A_wq.shape, BF16),
            pltpu.VMEM(A_wo.shape, BF16),
            pltpu.VMEM(B_w_gate.shape, BF16),
            pltpu.VMEM(B_w_up.shape, BF16),
            pltpu.VMEM(B_w_down.shape, BF16),
            pltpu.VMEM((NSLOT, CHUNK, Dh), BF16),
            pltpu.VMEM((NSLOT, CHUNK, Dh), BF16),
            pltpu.VMEM((B, M, D), F32),
            pltpu.VMEM((B, M, D), F32),
            pltpu.VMEM((M, D), F32),
            pltpu.SemaphoreType.DMA((2, NSLOT)),
            pltpu.SemaphoreType.DMA((len(TAIL_CUTS),)),
        ],
        compiler_params=pltpu.CompilerParams(vmem_limit_bytes=64 * 1024 * 1024),
    )(A_x.reshape(B, D), A_k_cache, A_v_cache, A_wq, A_wo,
      B_w_r, B_w_gate, B_w_up, B_w_down)
    return out.reshape(A_x.shape)
```
